```python
import os as _os
_os.environ.setdefault("JAX_PLATFORMS", "cpu")
import jax
import jax.numpy as jnp

def _softmax(x, axis=-1):
    return jax.nn.softmax(x, axis=axis)
def _gelu(x):
    return jax.nn.gelu(x, approximate=True)
def _silu(x):
    return jax.nn.silu(x)
def _sigmoid(x):
    return jax.nn.sigmoid(x)
def _layernorm(x, axis=-1, eps=1e-5):
    m = jnp.mean(x, axis=axis, keepdims=True)
    v = jnp.var(x, axis=axis, keepdims=True)
    return (x - m) / jnp.sqrt(v + eps)
def _scatter_add(tgt, idx, src, axis=0):
    return tgt.at[idx].add(src)
def _segment_sum(src, seg, n):
    return jax.ops.segment_sum(src, seg, n)
class _Rng:
    def __init__(self, key):
        self._k = key
    def _next(self):
        self._k, sub = jax.random.split(self._k)
        return sub
    def normal(self, shape):
        return jax.random.normal(self._next(), shape, dtype=jnp.bfloat16)
    def randint(self, lo, hi, shape):
        return jax.random.randint(self._next(), shape, lo, hi, dtype=jnp.int32)
    def uniform(self, shape, lo=0.0, hi=1.0):
        return jax.random.uniform(self._next(), shape, jnp.bfloat16, lo, hi)
    def permutation(self, n):
        return jax.random.permutation(self._next(), n)


kernel_name = 'concat_heads__gqa_block_cached__gqa_block_cached__near_ridge'

def setup_inputs():
    _rng = _Rng(jax.random.key(int.from_bytes(__import__("os").urandom(4), "little")))
    _w = (lambda a: (lambda t: t.astype(jnp.bfloat16) if jnp.issubdtype(t.dtype, jnp.floating) else t)(jnp.asarray(a)))
    def _A_setup():
        B, Sq, D = 16, 144, 448
        Hq, Hkv, Sk, Dh = 16, 8, 1024, 256
        assert Hq % Hkv == 0, (Hq, Hkv)
        return {
            "x": _w((lambda *s: _rng.normal(s) * 0.8)(B, Sq, D)),
            "k_cache": _w((lambda *s: _rng.normal(s) * 0.8)(B, Hkv, Sk, Dh)),
            "v_cache": _w((lambda *s: _rng.normal(s) * 0.05)(B, Hkv, Sk, Dh)),
            "wq": _w((lambda *s: _rng.normal(s) * 0.8)(D, Hq * Dh) * (D ** -0.5)),
            "wo": _w((lambda *s: _rng.normal(s) * 0.05)(Hq * Dh, D) * ((Hq * Dh) ** -0.5)),
        }
    _A_in = _A_setup()

    def _B_setup():
        B, Sq, D = 16, 144, 448
        Hq, Hkv, Sk, Dh = 16, 8, 1024, 256
        assert Hq % Hkv == 0, (Hq, Hkv)
        return {
            "x": _w((lambda *s: _rng.normal(s) * 0.8)(B, Sq, D)),
            "k_cache": _w((lambda *s: _rng.normal(s) * 0.8)(B, Hkv, Sk, Dh)),
            "v_cache": _w((lambda *s: _rng.normal(s) * 0.05)(B, Hkv, Sk, Dh)),
            "wq": _w((lambda *s: _rng.normal(s) * 0.8)(D, Hq * Dh) * (D ** -0.5)),
            "wo": _w((lambda *s: _rng.normal(s) * 0.05)(Hq * Dh, D) * ((Hq * Dh) ** -0.5)),
        }
    _B_in = _B_setup()

    return {
        "A_x": _A_in["x"],
        "A_k_cache": _A_in["k_cache"],
        "A_v_cache": _A_in["v_cache"],
        "A_wq": _A_in["wq"],
        "A_wo": _A_in["wo"],
        "B_x": _B_in["x"],
        "B_k_cache": _B_in["k_cache"],
        "B_v_cache": _B_in["v_cache"],
        "B_wq": _B_in["wq"],
        "B_wo": _B_in["wo"],
    }

def reference(A_x, A_k_cache, A_v_cache, A_wq, A_wo, B_x, B_k_cache, B_v_cache, B_wq, B_wo):
    def _A_ref(x, k_cache, v_cache, wq, wo):
        B, Sq, D = x.shape
        Hq, Dh = 16, 256
        Hkv = k_cache.shape[1]
        rep = Hq // Hkv
        q = (lambda x, *d: x.transpose(*d))((x @ wq).reshape(B, Sq, Hq, Dh), 0, 2, 1, 3)
        k = jnp.repeat(k_cache, rep, axis=1)
        v = jnp.repeat(v_cache, rep, axis=1)
        scores = jnp.einsum("bhqd,bhkd->bhqk", q, k) * (Dh ** -0.5)
        p = _softmax(scores, axis=-1)
        o = jnp.einsum("bhqk,bhkd->bhqd", p, v)
        return (lambda x, *d: x.transpose(*d))(o, 0, 2, 1, 3).reshape(B, Sq, Hq * Dh) @ wo

    def _B_ref(x, k_cache, v_cache, wq, wo):
        B, Sq, D = x.shape
        Hq, Dh = 16, 256
        Hkv = k_cache.shape[1]
        rep = Hq // Hkv
        q = (lambda x, *d: x.transpose(*d))((x @ wq).reshape(B, Sq, Hq, Dh), 0, 2, 1, 3)
        k = jnp.repeat(k_cache, rep, axis=1)
        v = jnp.repeat(v_cache, rep, axis=1)
        scores = jnp.einsum("bhqd,bhkd->bhqk", q, k) * (Dh ** -0.5)
        p = _softmax(scores, axis=-1)
        o = jnp.einsum("bhqk,bhkd->bhqd", p, v)
        return (lambda x, *d: x.transpose(*d))(o, 0, 2, 1, 3).reshape(B, Sq, Hq * Dh) @ wo

    a = _A_ref(A_x, A_k_cache, A_v_cache, A_wq, A_wo)
    b = _B_ref(B_x, B_k_cache, B_v_cache, B_wq, B_wo)
    return jnp.concatenate([a, b], axis=-1)
```

```python
import jax
import jax.numpy as jnp
import numpy as np
import jax.experimental.pallas as pl
import jax.experimental.pallas.tpu as pltpu

B, SQ, D, HQ, HKV, SK, DH = 16, 144, 448, 16, 8, 1024, 256
HW = (HQ // HKV) * DH
T = B * SQ
HALF = T // 2
RC = D // 4
KC = SK // 2
U = 4
NI = B // U
NBODY = HKV * NI
NSET = 3
X_STAGES = ((0, 0, 4), (0, 4, 9), (0, 9, 16), (1, 0, 8), (1, 8, 16))
OUT_CHUNKS = (9, 5, 3, 1)
Q_SCALE = float(np.log2(np.e)) * DH ** -0.5
NT = (((1,), (1,)), ((), ()))
F32, BF16 = jnp.float32, jnp.bfloat16


def _kernel(xa, ka, va, wqa, woa, xb, kb, vb, wqb, wob, out,
            x_s, wq_s, wo_s, k_s, v_s, q0_s, q_s, o_s, acc, stage, p_s,
            sem_kv, sem_x, sem_wq, sem_wo, sem_o):
    xs, ks, vs, wqs, wos = (xa, xb), (ka, kb), (va, vb), (wqa, wqb), (woa, wob)

    def kv_copies(g, slot):
        h, b0 = g // NI, (g % NI) * U
        cs = []
        for br in range(2):
            cs.append(pltpu.make_async_copy(ks[br].at[pl.ds(b0, U), h], k_s.at[br, slot], sem_kv.at[0, br, slot]))
            cs.append(pltpu.make_async_copy(vs[br].at[pl.ds(b0, U), h], v_s.at[br, slot], sem_kv.at[1, br, slot]))
        return cs

    def wq_copy(br, h):
        cols = pl.ds(pl.multiple_of(h * HW, HW), HW)
        return pltpu.make_async_copy(wqs[br].at[:, cols], wq_s.at[br, h], sem_wq.at[br, h])

    def wo_copies(br):
        return [pltpu.make_async_copy(wos[br].at[:, h * HW:(h + 1) * HW], wo_s.at[br, h], sem_wo.at[br])
                for h in range(HKV)]

    def x_copy(br, b0, b1):
        return pltpu.make_async_copy(xs[br].at[b0:b1], x_s.at[br, b0:b1], sem_x.at[br])

    def q_buf(br, h, b):
        return q0_s.at[br, b] if isinstance(h, int) and h == 0 else q_s.at[h - 1, br, b]

    def q_proj(br, h, b):
        q = jnp.dot(x_s[br, b], wq_s[br, h], preferred_element_type=F32) * Q_SCALE
        q = q.astype(BF16)
        dst = q_buf(br, h, b)
        dst[:SQ, :] = q[:, :DH]
        dst[SQ:, :] = q[:, DH:]

    def scores(br, h, b, slot, u, i, split):
        n = 2 * SQ // split
        alphas, invs = [], []
        for r in range(split):
            rows = slice(r * n, (r + 1) * n)
            ms, ls = [], []
            for j in range(2):
                keys = slice(j * KC, (j + 1) * KC)
                s = jax.lax.dot_general(q_buf(br, h, b)[rows, :], k_s[br, slot, u, keys, :], NT,
                                        preferred_element_type=F32)
                m = jnp.max(s, axis=-1, keepdims=True)
                if j > 0:
                    m = jnp.maximum(m, ms[-1])
                p = jnp.exp2(s - m)
                ls.append(jnp.sum(p, axis=-1, keepdims=True))
                ms.append(m)
                p_s[i, rows, keys] = p.astype(BF16)
            alpha = jnp.exp2(ms[0] - ms[1])
            alphas.append(alpha)
            invs.append(1.0 / (alpha * ls[0] + ls[1]))
        return jnp.concatenate(alphas, axis=0), jnp.concatenate(invs, axis=0)

    def values(br, h, b, slot, u, i, split, alpha, inv):
        n = 2 * SQ // split
        outs = []
        for r in range(split):
            rows = slice(r * n, (r + 1) * n)
            o = jnp.dot(p_s[i, rows, :KC], v_s[br, slot, u, :KC, :], preferred_element_type=F32) * alpha[rows]
            o = o + jnp.dot(p_s[i, rows, KC:], v_s[br, slot, u, KC:, :], preferred_element_type=F32)
            outs.append((o * inv[rows]).astype(BF16))
        o = jnp.concatenate(outs, axis=0)
        tokens = pl.ds(pl.multiple_of(b * SQ, SQ), SQ)
        dst = o_s.at[h & 1]
        dst[br, tokens, :DH] = o[:SQ]
        dst[br, tokens, DH:] = o[SQ:]

    def out_proj_unit(h, j):
        br, r, half = j & 1, (j >> 1) & 3, j >> 3
        w = wo_s[br, h, pl.ds(pl.multiple_of(r * RC, RC), RC), :]
        rows = pl.ds(pl.multiple_of(br * D + r * RC, RC), RC)
        o = o_s.at[h & 1][br, pl.ds(pl.multiple_of(half * HALF, HALF), HALF), :]
        acc[half, rows, :] += jax.lax.dot_general(w, o, NT, preferred_element_type=F32)

    wq_copy(0, 0).start()
    x_copy(*X_STAGES[0]).start()
    acc[...] = jnp.zeros_like(acc)
    for si, (br, b0, b1) in enumerate(X_STAGES):
        if b0 == 0:
            wq_copy(br, 0).wait()
        x_copy(br, b0, b1).wait()
        if si + 1 < len(X_STAGES):
            if X_STAGES[si + 1][1] == 0:
                wq_copy(X_STAGES[si + 1][0], 0).start()
            x_copy(*X_STAGES[si + 1]).start()
        if si >= len(X_STAGES) - 2:
            for br2 in range(2):
                wq_copy(br2, si - len(X_STAGES) + 3).start()
        for b in range(b0, b1):
            q_proj(br, 0, b)

    @pl.loop(1, HKV - 1)
    def _(h):
        for br in range(2):
            wq_copy(br, h).wait()

        @pl.when(h == 1)
        def _():
            for hh in range(3, HKV):
                for br in range(2):
                    wq_copy(br, hh).start()

        @pl.when(h == 2)
        def _():
            for br in range(2):
                for c in wo_copies(br):
                    c.start()

        for g in range(NSET - 1):
            @pl.when(h == 3 + g)
            def _():
                for c in kv_copies(g, g):
                    c.start()

        for br in range(2):
            for b in range(B):
                q_proj(br, h, b)

    for br in range(2):
        wq_copy(br, HKV - 1).wait()
        for c in wo_copies(br):
            c.wait()

    def body(g, slot, first):
        for c in kv_copies(g, slot):
            c.wait()
        nxt = g + (NSET - 1)
        nxt_slot = jnp.where(slot == 0, NSET - 1, slot - 1)

        @pl.when(nxt < NBODY)
        def _():
            for c in kv_copies(nxt, nxt_slot):
                c.start()

        for u in range(U):
            b = (g % NI) * U + u
            ia, ib = 2 * (u % 2), 2 * (u % 2) + 1
            if first:
                ca = scores(0, 0, b, slot, u, ia, 2)
                q_proj(0, HKV - 1, b)
                cb = scores(1, 0, b, slot, u, ib, 2)
                q_proj(1, HKV - 1, b)
                values(0, 0, b, slot, u, ia, 2, *ca)
                values(1, 0, b, slot, u, ib, 2, *cb)
            else:
                h = g // NI
                ca = scores(0, h, b, slot, u, ia, 1)
                cb = scores(1, h, b, slot, u, ib, 1)
                out_proj_unit(h - 1, b)
                values(0, h, b, slot, u, ia, 1, *ca)
                values(1, h, b, slot, u, ib, 1, *cb)
        return jnp.where(slot == NSET - 1, 0, slot + 1)

    slot = jax.lax.fori_loop(0, NI, lambda g, s: body(g, s, True), 0)
    slot = jax.lax.fori_loop(NI, NBODY, lambda g, s: body(g, s, False), slot)

    last_h = HKV - 1

    def emit(tile, r):
        stage[tile * 128:(tile + 1) * 128, :] = r.T.astype(BF16)

    copies = []
    t0 = 0
    for c, n in enumerate(OUT_CHUNKS):
        lo, hi = max(t0 - 1, 0), (t0 + n if c == len(OUT_CHUNKS) - 1 else t0 + n - 1)
        cp = pltpu.make_async_copy(stage.at[lo * 128:hi * 128], out.at[lo * 128:hi * 128], sem_o.at[c])

        @pl.when(slot >= -c)
        def _():
            if c > 0:
                tile = t0 - 1
                emit(tile, acc[tile // 9, :, (tile % 9) * 128:(tile % 9 + 1) * 128])
            for tile in range(t0, t0 + n):
                parts = []
                for br in range(2):
                    o = o_s[last_h & 1, br, tile * 128:(tile + 1) * 128, :]
                    parts.append(jax.lax.dot_general(wo_s[br, last_h], o, NT, preferred_element_type=F32))
                half, off = tile // 9, (tile % 9) * 128
                r = jnp.concatenate(parts, axis=0) + acc[half, :, off:off + 128]
                if tile < hi:
                    emit(tile, r)
                else:
                    acc[half, :, off:off + 128] = r
            cp.start()

        copies.append(cp)
        t0 += n
    for cp in copies:
        cp.wait()


@jax.jit
def pallas_concat_heads__gqa_block_cached__gqa_block_cached__near_ridge_kernel(
    A_x: jax.Array,
    A_k_cache: jax.Array,
    A_v_cache: jax.Array,
    A_wq: jax.Array,
    A_wo: jax.Array,
    B_x: jax.Array,
    B_k_cache: jax.Array,
    B_v_cache: jax.Array,
    B_wq: jax.Array,
    B_wo: jax.Array,
):
    assert A_x.shape == B_x.shape == (B, SQ, D)
    assert A_k_cache.shape == B_k_cache.shape == (B, HKV, SK, DH)
    hbm = pl.BlockSpec(memory_space=pltpu.HBM)
    out = pl.pallas_call(
        _kernel,
        in_specs=[hbm] * 10,
        out_specs=hbm,
        out_shape=jax.ShapeDtypeStruct((T, 2 * D), BF16),
        scratch_shapes=[
            pltpu.VMEM((2, B, SQ, D), BF16),
            pltpu.VMEM((2, HKV, D, HW), BF16),
            pltpu.VMEM((2, HKV, D, HW), BF16),
            pltpu.VMEM((2, NSET, U, SK, DH), BF16),
            pltpu.VMEM((2, NSET, U, SK, DH), BF16),
            pltpu.VMEM((2, B, 2 * SQ, DH), BF16),
            pltpu.VMEM((HKV - 1, 2, B, 2 * SQ, DH), BF16),
            pltpu.VMEM((2, 2, T, HW), BF16),
            pltpu.VMEM((2, 2 * D, HALF), F32),
            pltpu.VMEM((T, 2 * D), BF16),
            pltpu.VMEM((4, 2 * SQ, SK), BF16),
            pltpu.SemaphoreType.DMA((2, 2, NSET)),
            pltpu.SemaphoreType.DMA((2,)),
            pltpu.SemaphoreType.DMA((2, HKV)),
            pltpu.SemaphoreType.DMA((2,)),
            pltpu.SemaphoreType.DMA((len(OUT_CHUNKS),)),
        ],
        compiler_params=pltpu.CompilerParams(vmem_limit_bytes=120 * 2**20, disable_bounds_checks=True),
    )(A_x, A_k_cache, A_v_cache, A_wq, A_wo.T, B_x, B_k_cache, B_v_cache, B_wq, B_wo.T)
    return out.reshape(B, SQ, 2 * D)
```

```python
import jax
import jax.numpy as jnp
import numpy as np
import jax.experimental.pallas as pl
import jax.experimental.pallas.tpu as pltpu

B, SQ, D, HQ, HKV, SK, DH = 16, 144, 448, 16, 8, 1024, 256
HW = (HQ // HKV) * DH
T = B * SQ
KC = SK // 2
U = 8
NI = B // U
NBODY = HKV * NI
UT = U * SQ // 128
U0 = 4
X_STAGES = ((0, 0, 4), (0, 4, 9), (0, 9, 16), (1, 0, 8), (1, 8, 16))
FIRST_ORDER = ("qa qb sa va sb vb", "sa sb va vb qa qb", "sa qa qb sb va vb", "qa sa sb qb va vb")
OUT_CHUNKS = (9, 5, 3, 1)
Q_SCALE = float(np.log2(np.e)) * DH ** -0.5
NT = (((1,), (1,)), ((), ()))
F32, BF16 = jnp.float32, jnp.bfloat16


def _kernel(xa, ka, va, wqa, woa, xb, kb, vb, wqb, wob, out,
            wo_s, k_s, v_s, q_s, o_s, acc, p_s,
            sem_kv, sem_x, sem_wq, sem_wo, sem_o):
    xs, ks, vs, wqs, wos = (xa, xb), (ka, kb), (va, vb), (wqa, wqb), (woa, wob)

    def kv_copies(g, slot):
        h, b0 = g // NI, (g % NI) * U
        cs = []
        for br in range(2):
            cs.append(pltpu.make_async_copy(ks[br].at[pl.ds(b0, U), h], k_s.at[br, slot], sem_kv.at[0, br, slot]))
            cs.append(pltpu.make_async_copy(vs[br].at[pl.ds(b0, U), h], v_s.at[br, slot], sem_kv.at[1, br, slot]))
        return cs

    def scores(br, q_ref, slot, u, split):
        n = 2 * SQ // split
        alphas, invs = [], []
        for r in range(split):
            rows = slice(r * n, (r + 1) * n)
            ms, ls = [], []
            for j in range(2):
                keys = slice(j * KC, (j + 1) * KC)
                s = jax.lax.dot_general(q_ref[rows, :], k_s[br, slot, u, keys, :], NT, preferred_element_type=F32)
                m = jnp.max(s, axis=-1, keepdims=True)
                if j > 0:
                    m = jnp.maximum(m, ms[-1])
                p = jnp.exp2(s - m)
                ls.append(jnp.sum(p, axis=-1, keepdims=True))
                ms.append(m)
                p_s[br, rows, keys] = p.astype(BF16)
            alpha = jnp.exp2(ms[0] - ms[1])
            alphas.append(alpha)
            invs.append(1.0 / (alpha * ls[0] + ls[1]))
        return jnp.concatenate(alphas, axis=0), jnp.concatenate(invs, axis=0)

    def values(br, h, b, slot, u, split, alpha, inv):
        n = 2 * SQ // split
        outs = []
        for r in range(split):
            rows = slice(r * n, (r + 1) * n)
            o = jnp.dot(p_s[br, rows, :KC], v_s[br, slot, u, :KC, :], preferred_element_type=F32) * alpha[rows]
            o = o + jnp.dot(p_s[br, rows, KC:], v_s[br, slot, u, KC:, :], preferred_element_type=F32)
            outs.append((o * inv[rows]).astype(BF16))
        o = jnp.concatenate(outs, axis=0)
        tokens = pl.ds(pl.multiple_of(b * SQ, SQ), SQ)
        dst = o_s.at[h & 1]
        dst[br, tokens, :DH] = o[:SQ]
        dst[br, tokens, DH:] = o[SQ:]

    def out_proj(h, b, u):
        i = b >> 3
        for unit in range(u * 2 * UT // U, (u + 1) * 2 * UT // U):
            tile, br = unit // 2, unit % 2
            o = o_s.at[h & 1][br, pl.ds(pl.multiple_of((i * UT + tile) * 128, 128), 128), :]
            acc[i, br * D:(br + 1) * D, tile * 128:(tile + 1) * 128] += jax.lax.dot_general(
                wo_s[br, h], o, NT, preferred_element_type=F32)

    def body(g, slot, compute):
        for c in kv_copies(g, slot):
            c.wait()
        compute(g, slot)

        @pl.when(g + 2 < NBODY)
        def _():
            for c in kv_copies(g + 2, slot):
                c.start()

        return jnp.where(slot == 1, 0, slot + 1)

    def first_head(x_s, wq_s, q0_s):
        def wq_copy(br, h):
            cols = pl.ds(pl.multiple_of(h * HW, HW), HW)
            return pltpu.make_async_copy(wqs[br].at[:, cols], wq_s.at[br, h], sem_wq.at[br, h])

        def wo_copies(br):
            return [pltpu.make_async_copy(wos[br].at[:, h * HW:(h + 1) * HW], wo_s.at[br, h], sem_wo.at[br])
                    for h in range(HKV)]

        def x_copy(br, b0, b1):
            return pltpu.make_async_copy(xs[br].at[b0:b1], x_s.at[br, b0:b1], sem_x.at[br])

        def q_proj(br, h, b, dst):
            q = jnp.dot(x_s[br, b], wq_s[br, h], preferred_element_type=F32) * Q_SCALE
            q = q.astype(BF16)
            dst[:SQ, :] = q[:, :DH]
            dst[SQ:, :] = q[:, DH:]

        wq_copy(0, 0).start()
        x_copy(*X_STAGES[0]).start()
        acc[...] = jnp.zeros_like(acc)
        for si, (br, b0, b1) in enumerate(X_STAGES):
            if b0 == 0:
                wq_copy(br, 0).wait()
            x_copy(br, b0, b1).wait()
            if si + 1 < len(X_STAGES):
                if X_STAGES[si + 1][1] == 0:
                    wq_copy(X_STAGES[si + 1][0], 0).start()
                x_copy(*X_STAGES[si + 1]).start()
            if si >= len(X_STAGES) - 2:
                for br2 in range(2):
                    wq_copy(br2, si - len(X_STAGES) + 3).start()
            for b in range(b0, b1):
                q_proj(br, 0, b, q0_s.at[br, b])

        @pl.loop(0, HKV - 2)
        def _(i):
            h = i + 1
            for br in range(2):
                wq_copy(br, h).wait()

            @pl.when(i == 0)
            def _():
                for hh in range(3, HKV):
                    for br in range(2):
                        wq_copy(br, hh).start()

            @pl.when(i == 1)
            def _():
                for br in range(2):
                    for c in wo_copies(br):
                        c.start()

            for g in range(2):
                @pl.when(i == 2 + 2 * g)
                def _():
                    for c in kv_copies(g, g):
                        c.start()

            for br in range(2):
                for b in range(B):
                    q_proj(br, h, b, q_s.at[h - 1, br, b])

        for br in range(2):
            wq_copy(br, HKV - 1).wait()
            for c in wo_copies(br):
                c.wait()

        def compute(g, slot):
            @pl.loop(0, U // U0)
            def _(k):
                for uu in range(U0):
                    b, u = g * U + k * U0 + uu, k * U0 + uu
                    scale = [None, None]
                    for op in FIRST_ORDER[uu].split():
                        br = "ab".index(op[1])
                        if op[0] == "s":
                            scale[br] = scores(br, q0_s.at[br, b], slot, u, 2)
                        elif op[0] == "v":
                            values(br, 0, b, slot, u, 2, *scale[br])
                        else:
                            q_proj(br, HKV - 1, b, q_s.at[HKV - 2, br, b])

        jax.lax.fori_loop(0, NI, lambda g, slot: body(g, slot, compute), 0)

    pl.run_scoped(
        first_head,
        pltpu.VMEM((2, B, SQ, D), BF16),
        pltpu.VMEM((2, HKV, D, HW), BF16),
        pltpu.VMEM((2, B, 2 * SQ, DH), BF16),
    )

    def compute(g, slot):
        for u in range(U):
            h, b = g // NI, (g % NI) * U + u
            sa = scores(0, q_s.at[h - 1, 0, b], slot, u, 1)
            sb = scores(1, q_s.at[h - 1, 1, b], slot, u, 1)
            out_proj(h - 1, b, u)
            values(0, h, b, slot, u, 1, *sa)
            values(1, h, b, slot, u, 1, *sb)

    slot = jax.lax.fori_loop(NI, NBODY, lambda g, slot: body(g, slot, compute), NI % 2)

    def write_back(stage):
        h = HKV - 1

        def emit(tile, r):
            stage[tile * 128:(tile + 1) * 128, :] = r.T.astype(BF16)

        copies = []
        t0 = 0
        for c, n in enumerate(OUT_CHUNKS):
            lo, hi = max(t0 - 1, 0), (t0 + n if c == len(OUT_CHUNKS) - 1 else t0 + n - 1)
            cp = pltpu.make_async_copy(stage.at[lo * 128:hi * 128], out.at[lo * 128:hi * 128], sem_o.at[c])

            @pl.when(slot >= -c)
            def _():
                if c > 0:
                    tile = t0 - 1
                    emit(tile, acc[tile // UT, :, (tile % UT) * 128:(tile % UT + 1) * 128])
                for tile in range(t0, t0 + n):
                    parts = []
                    for br in range(2):
                        o = o_s[h & 1, br, tile * 128:(tile + 1) * 128, :]
                        parts.append(jax.lax.dot_general(wo_s[br, h], o, NT, preferred_element_type=F32))
                    i, off = tile // UT, (tile % UT) * 128
                    r = jnp.concatenate(parts, axis=0) + acc[i, :, off:off + 128]
                    if tile < hi:
                        emit(tile, r)
                    else:
                        acc[i, :, off:off + 128] = r
                cp.start()

            copies.append(cp)
            t0 += n
        for cp in copies:
            cp.wait()

    pl.run_scoped(write_back, pltpu.VMEM((T, 2 * D), BF16))


@jax.jit
def pallas_concat_heads__gqa_block_cached__gqa_block_cached__near_ridge_kernel(
    A_x: jax.Array,
    A_k_cache: jax.Array,
    A_v_cache: jax.Array,
    A_wq: jax.Array,
    A_wo: jax.Array,
    B_x: jax.Array,
    B_k_cache: jax.Array,
    B_v_cache: jax.Array,
    B_wq: jax.Array,
    B_wo: jax.Array,
):
    assert A_x.shape == B_x.shape == (B, SQ, D)
    assert A_k_cache.shape == B_k_cache.shape == (B, HKV, SK, DH)
    hbm = pl.BlockSpec(memory_space=pltpu.HBM)
    out = pl.pallas_call(
        _kernel,
        in_specs=[hbm] * 10,
        out_specs=hbm,
        out_shape=jax.ShapeDtypeStruct((T, 2 * D), BF16),
        scratch_shapes=[
            pltpu.VMEM((2, HKV, D, HW), BF16),
            pltpu.VMEM((2, 2, U, SK, DH), BF16),
            pltpu.VMEM((2, 2, U, SK, DH), BF16),
            pltpu.VMEM((HKV - 1, 2, B, 2 * SQ, DH), BF16),
            pltpu.VMEM((2, 2, T, HW), BF16),
            pltpu.VMEM((NI, 2 * D, UT * 128), F32),
            pltpu.VMEM((2, 2 * SQ, SK), BF16),
            pltpu.SemaphoreType.DMA((2, 2, 2)),
            pltpu.SemaphoreType.DMA((2,)),
            pltpu.SemaphoreType.DMA((2, HKV)),
            pltpu.SemaphoreType.DMA((2,)),
            pltpu.SemaphoreType.DMA((len(OUT_CHUNKS),)),
        ],
        compiler_params=pltpu.CompilerParams(vmem_limit_bytes=120 * 2**20, disable_bounds_checks=True),
    )(A_x, A_k_cache, A_v_cache, A_wq, A_wo.T, B_x, B_k_cache, B_v_cache, B_wq, B_wo.T)
    return out.reshape(B, SQ, 2 * D)
```

```python
import jax
import jax.numpy as jnp
import numpy as np
import jax.experimental.pallas as pl
import jax.experimental.pallas.tpu as pltpu

B, SQ, D, HQ, HKV, SK, DH = 16, 144, 448, 16, 8, 1024, 256
HW = (HQ // HKV) * DH
T = B * SQ
KC = SK // 2
U = 8
NI = B // U
NBODY = HKV * NI
UT = U * SQ // 128
U0 = 4
X_STAGES = ((0, 0, 2), (0, 2, 5), (0, 5, 10), (0, 10, 16), (1, 0, 8), (1, 8, 16))
HPI = 2
FIRST_ORDER = ("qb sa qa sb va vb", "sa sb qa va qb vb", "sa qa sb va vb qb", "sa qa sb va qb vb")
OUT_CHUNKS = (9, 5, 3, 1)
Q_SCALE = float(np.log2(np.e)) * DH ** -0.5
NT = (((1,), (1,)), ((), ()))
F32, BF16 = jnp.float32, jnp.bfloat16


def _kernel(xa, ka, va, wqa, woa, xb, kb, vb, wqb, wob, out,
            wo_s, k_s, v_s, q_s, o_s, acc, p_s,
            sem_kv, sem_x, sem_wq, sem_wo, sem_o):
    xs, ks, vs, wqs, wos = (xa, xb), (ka, kb), (va, vb), (wqa, wqb), (woa, wob)

    def kv_copies(g, slot):
        h, b0 = g // NI, (g % NI) * U
        cs = []
        for br in range(2):
            cs.append(pltpu.make_async_copy(ks[br].at[pl.ds(b0, U), h], k_s.at[br, slot], sem_kv.at[0, br, slot]))
            cs.append(pltpu.make_async_copy(vs[br].at[pl.ds(b0, U), h], v_s.at[br, slot], sem_kv.at[1, br, slot]))
        return cs

    def scores(br, q_ref, slot, u, split):
        n = 2 * SQ // split
        alphas, invs = [], []
        for r in range(split):
            rows = slice(r * n, (r + 1) * n)
            ms, ls = [], []
            for j in range(2):
                keys = slice(j * KC, (j + 1) * KC)
                s = jax.lax.dot_general(q_ref[rows, :], k_s[br, slot, u, keys, :], NT, preferred_element_type=F32)
                m = jnp.max(s, axis=-1, keepdims=True)
                if j > 0:
                    m = jnp.maximum(m, ms[-1])
                p = jnp.exp2(s - m)
                ls.append(jnp.sum(p, axis=-1, keepdims=True))
                ms.append(m)
                p_s[br, rows, keys] = p.astype(BF16)
            alpha = jnp.exp2(ms[0] - ms[1])
            alphas.append(alpha)
            invs.append(1.0 / (alpha * ls[0] + ls[1]))
        return jnp.concatenate(alphas, axis=0), jnp.concatenate(invs, axis=0)

    def values(br, h, b, slot, u, split, alpha, inv):
        n = 2 * SQ // split
        outs = []
        for r in range(split):
            rows = slice(r * n, (r + 1) * n)
            o = jnp.dot(p_s[br, rows, :KC], v_s[br, slot, u, :KC, :], preferred_element_type=F32) * alpha[rows]
            o = o + jnp.dot(p_s[br, rows, KC:], v_s[br, slot, u, KC:, :], preferred_element_type=F32)
            outs.append((o * inv[rows]).astype(BF16))
        o = jnp.concatenate(outs, axis=0)
        tokens = pl.ds(pl.multiple_of(b * SQ, SQ), SQ)
        dst = o_s.at[h & 1]
        dst[br, tokens, :DH] = o[:SQ]
        dst[br, tokens, DH:] = o[SQ:]

    def out_proj(h, b, u):
        i = b >> 3
        for unit in range(u * 2 * UT // U, (u + 1) * 2 * UT // U):
            tile, br = unit // 2, unit % 2
            o = o_s.at[h & 1][br, pl.ds(pl.multiple_of((i * UT + tile) * 128, 128), 128), :]
            acc[i, br * D:(br + 1) * D, tile * 128:(tile + 1) * 128] += jax.lax.dot_general(
                wo_s[br, h], o, NT, preferred_element_type=F32)

    assert U == 8 and (HKV - 2) % HPI == 0 and sum(OUT_CHUNKS) * 128 == T

    def body(g, slot, compute):
        for c in kv_copies(g, slot):
            c.wait()
        compute(g, slot)

        @pl.when(g + 2 < NBODY)
        def _():
            for c in kv_copies(g + 2, slot):
                c.start()

        return jnp.where(slot == 1, 0, slot + 1)

    def first_head(x_s, wq_s, q0_s):
        def wq_copy(br, h):
            cols = pl.ds(pl.multiple_of(h * HW, HW), HW)
            return pltpu.make_async_copy(wqs[br].at[:, cols], wq_s.at[br, h], sem_wq.at[br, h])

        def wo_copies(br):
            return [pltpu.make_async_copy(wos[br].at[:, h * HW:(h + 1) * HW], wo_s.at[br, h], sem_wo.at[br])
                    for h in range(HKV)]

        def x_copy(si):
            br, b0, b1 = X_STAGES[si]
            return pltpu.make_async_copy(xs[br].at[b0:b1], x_s.at[br, b0:b1], sem_x.at[si])

        def q_proj(br, h, b, dst):
            q = jnp.dot(x_s[br, b], wq_s[br, h], preferred_element_type=F32) * Q_SCALE
            q = q.astype(BF16)
            dst[:SQ, :] = q[:, :DH]
            dst[SQ:, :] = q[:, DH:]

        def start_branch(br):
            for si, stage in enumerate(X_STAGES):
                if stage[0] == br:
                    if stage[1] == 0:
                        wq_copy(br, 0).start(priority=min(si, 1))
                    x_copy(si).start(priority=min(si, 1))

        start_branch(0)
        acc[...] = jnp.zeros_like(acc)
        for si, (br, b0, b1) in enumerate(X_STAGES):
            if b0 == 0:
                wq_copy(br, 0).wait()
            x_copy(si).wait()
            if si == 1:
                start_branch(1)
            if si == len(X_STAGES) - 1:
                for h in range(1, HKV):
                    for br2 in range(2):
                        wq_copy(br2, h).start()
            for b in range(b0, b1):
                q_proj(br, 0, b, q0_s.at[br, b])

        steps = (HKV - 2) // HPI

        @pl.loop(0, steps)
        def _(i):
            heads = [1 + HPI * i + j for j in range(HPI)]
            for h in heads:
                for br in range(2):
                    wq_copy(br, h).wait()

            @pl.when(i == 0)
            def _():
                for br in range(2):
                    for c in wo_copies(br):
                        c.start()

            for g in range(2):
                @pl.when(i == steps - 2 + g)
                def _():
                    for c in kv_copies(g, g):
                        c.start()

            for h in heads:
                for br in range(2):
                    for b in range(B):
                        q_proj(br, h, b, q_s.at[h - 1, br, b])

        for br in range(2):
            wq_copy(br, HKV - 1).wait()
            for c in wo_copies(br):
                c.wait()

        def compute(g, slot):
            @pl.loop(0, U // U0)
            def _(k):
                for uu in range(U0):
                    b, u = g * U + k * U0 + uu, k * U0 + uu
                    scale = [None, None]
                    for op in FIRST_ORDER[uu].split():
                        br = "ab".index(op[1])
                        if op[0] == "s":
                            scale[br] = scores(br, q0_s.at[br, b], slot, u, 2)
                        elif op[0] == "v":
                            values(br, 0, b, slot, u, 2, *scale[br])
                        else:
                            q_proj(br, HKV - 1, b, q_s.at[HKV - 2, br, b])

        jax.lax.fori_loop(0, NI, lambda g, slot: body(g, slot, compute), 0)

    pl.run_scoped(
        first_head,
        pltpu.VMEM((2, B, SQ, D), BF16),
        pltpu.VMEM((2, HKV, D, HW), BF16),
        pltpu.VMEM((2, B, 2 * SQ, DH), BF16),
    )

    def compute(g, slot):
        for u in range(U):
            h, b = g // NI, (g % NI) * U + u
            sa = scores(0, q_s.at[h - 1, 0, b], slot, u, 1)
            sb = scores(1, q_s.at[h - 1, 1, b], slot, u, 1)
            out_proj(h - 1, b, u)
            values(0, h, b, slot, u, 1, *sa)
            values(1, h, b, slot, u, 1, *sb)

    slot = jax.lax.fori_loop(NI, NBODY, lambda g, slot: body(g, slot, compute), NI % 2)

    def write_back(stage):
        h = HKV - 1

        def emit(tile, r):
            stage[tile * 128:(tile + 1) * 128, :] = r.T.astype(BF16)

        copies = []
        t0 = 0
        for c, n in enumerate(OUT_CHUNKS):
            lo, hi = max(t0 - 1, 0), (t0 + n if c == len(OUT_CHUNKS) - 1 else t0 + n - 1)
            cp = pltpu.make_async_copy(stage.at[lo * 128:hi * 128], out.at[lo * 128:hi * 128], sem_o.at[c])

            @pl.when(slot >= -c)
            def _():
                if c > 0:
                    tile = t0 - 1
                    emit(tile, acc[tile // UT, :, (tile % UT) * 128:(tile % UT + 1) * 128])
                for tile in range(t0, t0 + n):
                    parts = []
                    for br in range(2):
                        o = o_s[h & 1, br, tile * 128:(tile + 1) * 128, :]
                        parts.append(jax.lax.dot_general(wo_s[br, h], o, NT, preferred_element_type=F32))
                    i, off = tile // UT, (tile % UT) * 128
                    r = jnp.concatenate(parts, axis=0) + acc[i, :, off:off + 128]
                    if tile < hi:
                        emit(tile, r)
                    else:
                        acc[i, :, off:off + 128] = r
                cp.start()

            copies.append(cp)
            t0 += n
        for cp in copies:
            cp.wait()

    pl.run_scoped(write_back, pltpu.VMEM((T, 2 * D), BF16))


@jax.jit
def pallas_concat_heads__gqa_block_cached__gqa_block_cached__near_ridge_kernel(
    A_x: jax.Array,
    A_k_cache: jax.Array,
    A_v_cache: jax.Array,
    A_wq: jax.Array,
    A_wo: jax.Array,
    B_x: jax.Array,
    B_k_cache: jax.Array,
    B_v_cache: jax.Array,
    B_wq: jax.Array,
    B_wo: jax.Array,
):
    assert A_x.shape == B_x.shape == (B, SQ, D)
    assert A_k_cache.shape == B_k_cache.shape == (B, HKV, SK, DH)
    hbm = pl.BlockSpec(memory_space=pltpu.HBM)
    out = pl.pallas_call(
        _kernel,
        in_specs=[hbm] * 10,
        out_specs=hbm,
        out_shape=jax.ShapeDtypeStruct((T, 2 * D), BF16),
        scratch_shapes=[
            pltpu.VMEM((2, HKV, D, HW), BF16),
            pltpu.VMEM((2, 2, U, SK, DH), BF16),
            pltpu.VMEM((2, 2, U, SK, DH), BF16),
            pltpu.VMEM((HKV - 1, 2, B, 2 * SQ, DH), BF16),
            pltpu.VMEM((2, 2, T, HW), BF16),
            pltpu.VMEM((NI, 2 * D, UT * 128), F32),
            pltpu.VMEM((2, 2 * SQ, SK), BF16),
            pltpu.SemaphoreType.DMA((2, 2, 2)),
            pltpu.SemaphoreType.DMA((len(X_STAGES),)),
            pltpu.SemaphoreType.DMA((2, HKV)),
            pltpu.SemaphoreType.DMA((2,)),
            pltpu.SemaphoreType.DMA((len(OUT_CHUNKS),)),
        ],
        compiler_params=pltpu.CompilerParams(vmem_limit_bytes=120 * 2**20, disable_bounds_checks=True),
    )(A_x, A_k_cache, A_v_cache, A_wq, A_wo.T, B_x, B_k_cache, B_v_cache, B_wq, B_wo.T)
    return out.reshape(B, SQ, 2 * D)
```
